```python
import os as _os
_os.environ.setdefault("JAX_PLATFORMS", "cpu")
import jax
import jax.numpy as jnp

def _softmax(x, axis=-1):
    return jax.nn.softmax(x, axis=axis)
def _gelu(x):
    return jax.nn.gelu(x, approximate=True)
def _silu(x):
    return jax.nn.silu(x)
def _sigmoid(x):
    return jax.nn.sigmoid(x)
def _layernorm(x, axis=-1, eps=1e-5):
    m = jnp.mean(x, axis=axis, keepdims=True)
    v = jnp.var(x, axis=axis, keepdims=True)
    return (x - m) / jnp.sqrt(v + eps)
def _scatter_add(tgt, idx, src, axis=0):
    return tgt.at[idx].add(src)
def _segment_sum(src, seg, n):
    return jax.ops.segment_sum(src, seg, n)
class _Rng:
    def __init__(self, key):
        self._k = key
    def _next(self):
        self._k, sub = jax.random.split(self._k)
        return sub
    def normal(self, shape):
        return jax.random.normal(self._next(), shape, dtype=jnp.bfloat16)
    def randint(self, lo, hi, shape):
        return jax.random.randint(self._next(), shape, lo, hi, dtype=jnp.int32)
    def uniform(self, shape, lo=0.0, hi=1.0):
        return jax.random.uniform(self._next(), shape, jnp.bfloat16, lo, hi)
    def permutation(self, n):
        return jax.random.permutation(self._next(), n)


kernel_name = 'gated_mix__gqa_block_cached__dense_activation_squared_relu__decode'

def setup_inputs():
    _rng = _Rng(jax.random.key(int.from_bytes(__import__("os").urandom(4), "little")))
    _w = (lambda a: (lambda t: t.astype(jnp.bfloat16) if jnp.issubdtype(t.dtype, jnp.floating) else t)(jnp.asarray(a)))
    def _A_setup():
        B, Sq, D = 4, 1, 512
        Hq, Hkv, Sk, Dh = 32, 8, 4096, 128
        assert Hq % Hkv == 0, (Hq, Hkv)
        return {
            "x": _w((lambda *s: _rng.normal(s) * 0.05)(B, Sq, D)),
            "k_cache": _w((lambda *s: _rng.normal(s) * 3.2)(B, Hkv, Sk, Dh)),
            "v_cache": _w((lambda *s: _rng.normal(s) * 1.6)(B, Hkv, Sk, Dh)),
            "wq": _w((lambda *s: _rng.normal(s) * 3.2)(D, Hq * Dh) * (D ** -0.5)),
            "wo": _w((lambda *s: _rng.normal(s) * 1.6)(Hq * Dh, D) * ((Hq * Dh) ** -0.5)),
        }
    _A_in = _A_setup()

    def _B_setup():
        B, S, D, F = 4, 1, 512, 1792
        return {
            "x": _w((lambda *s: _rng.normal(s) * 0.05)(B, S, D)),
            "w1": _w((lambda *s: _rng.normal(s) * 0.1)(D, F)),
            "b1": _w((lambda *s: _rng.normal(s) * 0.05)(F)),
            "w2": _w((lambda *s: _rng.normal(s) * 0.05)(F, D)),
            "b2": _w((lambda *s: _rng.normal(s) * 0.05)(D)),
        }
    _B_in = _B_setup()

    return {
        "A_x": _A_in["x"],
        "A_k_cache": _A_in["k_cache"],
        "A_v_cache": _A_in["v_cache"],
        "A_wq": _A_in["wq"],
        "A_wo": _A_in["wo"],
        "B_x": _B_in["x"],
        "B_w1": _B_in["w1"],
        "B_b1": _B_in["b1"],
        "B_w2": _B_in["w2"],
        "B_b2": _B_in["b2"],
        "gate_w": _w((lambda *s: _rng.normal(s) * 0.05)(512) * 16.0),
    }

def reference(A_x, A_k_cache, A_v_cache, A_wq, A_wo, B_x, B_w1, B_b1, B_w2, B_b2, gate_w):
    def _A_ref(x, k_cache, v_cache, wq, wo):
        B, Sq, D = x.shape
        Hq, Dh = 32, 128
        Hkv = k_cache.shape[1]
        rep = Hq // Hkv
        q = (lambda x, *d: x.transpose(*d))((x @ wq).reshape(B, Sq, Hq, Dh), 0, 2, 1, 3)
        k = jnp.repeat(k_cache, rep, axis=1)
        v = jnp.repeat(v_cache, rep, axis=1)
        scores = jnp.einsum("bhqd,bhkd->bhqk", q, k) * (Dh ** -0.5)
        p = _softmax(scores, axis=-1)
        o = jnp.einsum("bhqk,bhkd->bhqd", p, v)
        return (lambda x, *d: x.transpose(*d))(o, 0, 2, 1, 3).reshape(B, Sq, Hq * Dh) @ wo

    def _B_ref(x, w1, b1, w2, b2):
        h = jnp.einsum("bsd,df->bsf", x, w1) + b1
        zero = jnp.zeros_like(h)
        r = jnp.where(h > zero, h, zero)
        h = r * r
        out = jnp.einsum("bsf,fd->bsd", h, w2) + b2
        return out

    x = A_x
    g = _sigmoid((x * gate_w).sum(-1, keepdims=True))
    a = _A_ref(x, A_k_cache, A_v_cache, A_wq, A_wo)
    b = _B_ref(x, B_w1, B_b1, B_w2, B_b2)
    return g * a + (1 - g) * b
```

```python
import jax
import jax.numpy as jnp
import jax.experimental.pallas as pl
import jax.experimental.pallas.tpu as pltpu

_B, _D = 4, 512
_HQ, _HKV, _SK, _DH = 32, 8, 4096, 128
_REP = _HQ // _HKV
_F = 1792
_NBH = _B * _HKV
_LANES = 128

_KV_CHUNKS = (4, 4, 4, 4, 4, 4, 4, 4)
_WO_CHUNKS = (1024, 1024, 1024, 512, 256, 128, 128)
_WINDOW = 3


def _offsets(sizes):
    return [sum(sizes[:j]) for j in range(len(sizes))]


def _kernel(x_hbm, k_hbm, v_hbm, wq_hbm, wo_hbm, w1_hbm, b1_hbm, w2_hbm, b2_hbm, gw_hbm,
            o_ref,
            x_v, b1_v, b2_v, gw_v, wq_v, wo_v, w1_v, w2_v, k_v, v_v, qp_s, qt_s, ot_s,
            sem_s, sem_k, sem_v, sem_wo):
    f32, bf16 = jnp.float32, jnp.bfloat16
    n_kv, n_wo = len(_KV_CHUNKS), len(_WO_CHUNKS)
    kv_off, wo_off = _offsets(_KV_CHUNKS), _offsets(_WO_CHUNKS)

    c_x = pltpu.make_async_copy(x_hbm, x_v, sem_s.at[0])
    c_wq = pltpu.make_async_copy(wq_hbm, wq_v, sem_s.at[1])
    c_w1 = pltpu.make_async_copy(w1_hbm, w1_v, sem_s.at[2])
    c_w2 = pltpu.make_async_copy(w2_hbm, w2_v, sem_s.at[3])
    c_b1 = pltpu.make_async_copy(b1_hbm, b1_v, sem_s.at[4])
    c_b2 = pltpu.make_async_copy(b2_hbm, b2_v, sem_s.at[5])
    c_gw = pltpu.make_async_copy(gw_hbm, gw_v, sem_s.at[6])
    c_k, c_v = [], []
    for c in range(n_kv):
        sl = pl.ds(kv_off[c], _KV_CHUNKS[c])
        c_k.append(pltpu.make_async_copy(k_hbm.at[sl], k_v.at[sl], sem_k.at[c]))
        c_v.append(pltpu.make_async_copy(v_hbm.at[sl], v_v.at[sl], sem_v.at[c]))
    c_wo = []
    for j in range(n_wo):
        sl = pl.ds(wo_off[j], _WO_CHUNKS[j])
        c_wo.append(pltpu.make_async_copy(wo_hbm.at[sl], wo_v.at[sl], sem_wo.at[j]))

    queue = [c_wq]
    for c in range(n_kv):
        queue += [c_k[c], c_v[c]]
    queue += [c_w1, c_w2] + c_wo
    position = {id(c): i for i, c in enumerate(queue)}
    issued = [0]

    def issue_upto(n):
        while issued[0] < min(n, len(queue)):
            queue[issued[0]].start()
            issued[0] += 1

    def wait(c):
        i = position[id(c)]
        issue_upto(i + 1)
        c.wait()
        issue_upto(i + 1 + _WINDOW)

    c_x.start()
    issue_upto(_WINDOW)
    c_gw.start()
    c_b1.start()
    c_b2.start()

    c_x.wait()
    x4 = x_v[...]
    xf = x4.astype(f32)
    wait(c_wq)
    q = jnp.dot(x4, wq_v[...], preferred_element_type=f32)
    for j in range(_HQ):
        qp_s[pl.ds(j * 8, _B), :] = q[:, j * _DH:(j + 1) * _DH]
    zeros = jnp.zeros((8 - _REP, _DH), f32)
    for b in range(_B):
        for h in range(_HKV):
            i = b * _HKV + h
            qt_s[i, 0:_REP, :] = qp_s[pl.ds(h * _REP * 8 + b, _REP, stride=8), :]
            qt_s[i, _REP:8, :] = zeros

    scale = _DH ** -0.5

    def head(i, carry):
        qh = qt_s[i].astype(bf16)
        s = jax.lax.dot_general(qh, k_v[i], (((1,), (1,)), ((), ())),
                                preferred_element_type=f32) * scale
        m = jnp.max(s, axis=1, keepdims=True)
        p = jnp.exp(s - m)
        l = jnp.sum(p, axis=1, keepdims=True)
        o = jnp.dot(p.astype(bf16), v_v[i], preferred_element_type=f32)
        ot_s[pl.ds(pl.multiple_of(i * 8, 8), 8), :] = o / l
        return carry

    for c in range(n_kv):
        wait(c_k[c])
        wait(c_v[c])
        jax.lax.fori_loop(kv_off[c], kv_off[c] + _KV_CHUNKS[c], head, 0)

    c_gw.wait()
    c_b1.wait()
    c_b2.wait()
    gw = gw_v[...].astype(f32)
    gsum = jnp.zeros((_B, 1), f32)
    for t in range(_D // _LANES):
        gsum = gsum + jnp.sum(xf[:, t * _LANES:(t + 1) * _LANES] * gw[t:t + 1, :],
                              axis=1, keepdims=True)
    g = jax.nn.sigmoid(gsum)
    wait(c_w1)
    hpre = jnp.dot(x4, w1_v[...], preferred_element_type=f32)
    b1 = b1_v[...].astype(f32)
    hs = []
    for t in range(_F // _LANES):
        ht = hpre[:, t * _LANES:(t + 1) * _LANES] + b1[t:t + 1, :]
        r = jnp.where(ht > 0, ht, 0.0)
        hs.append((r * r).astype(bf16))
    hh = jnp.concatenate(hs, axis=1)
    wait(c_w2)
    mlp = jnp.dot(hh, w2_v[...], preferred_element_type=f32)
    b2 = b2_v[...].astype(f32)
    mlp = mlp + jnp.concatenate([b2[t:t + 1, :] for t in range(_D // _LANES)], axis=1)
    mix_b = (1.0 - g) * mlp

    acc = jnp.zeros((_B, _D), f32)
    for j in range(n_wo):
        tiles = []
        for t in range(wo_off[j] // _DH, (wo_off[j] + _WO_CHUNKS[j]) // _DH):
            h, r = t // _REP, t % _REP
            tiles.append(ot_s[pl.ds(8 * h + r, _B, stride=8 * _HKV), :].astype(bf16))
        lhs = tiles[0] if len(tiles) == 1 else jnp.concatenate(tiles, axis=1)
        wait(c_wo[j])
        acc = acc + jnp.dot(lhs, wo_v[pl.ds(wo_off[j], _WO_CHUNKS[j]), :],
                            preferred_element_type=f32)
    o_ref[...] = (g * acc + mix_b).astype(o_ref.dtype)


@jax.jit
def pallas_gated_mix__gqa_block_cached__dense_activation_squared_relu__decode_kernel(
    A_x: jax.Array,
    A_k_cache: jax.Array,
    A_v_cache: jax.Array,
    A_wq: jax.Array,
    A_wo: jax.Array,
    B_x: jax.Array,
    B_w1: jax.Array,
    B_b1: jax.Array,
    B_w2: jax.Array,
    B_b2: jax.Array,
    gate_w: jax.Array,
):
    del B_x
    f32, bf16 = jnp.float32, jnp.bfloat16
    hbm = pl.BlockSpec(memory_space=pltpu.HBM)
    n_kv, n_wo = len(_KV_CHUNKS), len(_WO_CHUNKS)
    out = pl.pallas_call(
        _kernel,
        in_specs=[hbm] * 10,
        out_specs=pl.BlockSpec(memory_space=pltpu.VMEM),
        out_shape=jax.ShapeDtypeStruct((_B, _D), bf16),
        scratch_shapes=[
            pltpu.VMEM((_B, _D), bf16),
            pltpu.VMEM((_F // _LANES, _LANES), bf16),
            pltpu.VMEM((_D // _LANES, _LANES), bf16),
            pltpu.VMEM((_D // _LANES, _LANES), bf16),
            pltpu.VMEM((_D, _HQ * _DH), bf16),
            pltpu.VMEM((_HQ * _DH, _D), bf16),
            pltpu.VMEM((_D, _F), bf16),
            pltpu.VMEM((_F, _D), bf16),
            pltpu.VMEM((_NBH, _SK, _DH), bf16),
            pltpu.VMEM((_NBH, _SK, _DH), bf16),
            pltpu.VMEM((_HQ * 8 + 8, _DH), f32),
            pltpu.VMEM((_NBH, 8, _DH), f32),
            pltpu.VMEM((_NBH * 8 + 64, _DH), f32),
            pltpu.SemaphoreType.DMA((7,)),
            pltpu.SemaphoreType.DMA((n_kv,)),
            pltpu.SemaphoreType.DMA((n_kv,)),
            pltpu.SemaphoreType.DMA((n_wo,)),
        ],
        compiler_params=pltpu.CompilerParams(vmem_limit_bytes=100 * 1024 * 1024),
    )(
        A_x.reshape(_B, _D),
        A_k_cache.reshape(_NBH, _SK, _DH),
        A_v_cache.reshape(_NBH, _SK, _DH),
        A_wq,
        A_wo,
        B_w1,
        B_b1.reshape(_F // _LANES, _LANES),
        B_w2,
        B_b2.reshape(_D // _LANES, _LANES),
        gate_w.reshape(_D // _LANES, _LANES),
    )
    return out.reshape(_B, 1, _D)
```

```python
import jax
import jax.numpy as jnp
import jax.experimental.pallas as pl
import jax.experimental.pallas.tpu as pltpu

_B, _D = 4, 512
_HQ, _HKV, _SK, _DH = 32, 8, 4096, 128
_REP = _HQ // _HKV
_F = 1792
_NBH = _B * _HKV
_LANES = 128

_KV_CHUNKS = (4, 4, 4, 4, 4, 4, 4, 4)
_WO_CHUNKS = (1024, 1024, 1024, 512, 256, 128, 128)
_WINDOW = 4


def _offsets(sizes):
    return [sum(sizes[:j]) for j in range(len(sizes))]


def _body(x_hbm, k_hbm, v_hbm, wq_hbm, wo_hbm, w1_hbm, b1_hbm, w2_hbm, b2_hbm, gw_hbm,
          o_ref,
          x_v, b1_v, b2_v, gw_v, wq_v, wo_v, w1_v, w2_v, k_v, v_v, qp_s, qt_s, ot_s,
          sems):
    f32, bf16 = jnp.float32, jnp.bfloat16
    n_kv, n_wo = len(_KV_CHUNKS), len(_WO_CHUNKS)
    kv_off, wo_off = _offsets(_KV_CHUNKS), _offsets(_WO_CHUNKS)

    plan = [("wq", wq_hbm, wq_v)]
    for c in range(n_kv):
        sl = pl.ds(kv_off[c], _KV_CHUNKS[c])
        plan.append((("k", c), k_hbm.at[sl], k_v.at[sl]))
        plan.append((("v", c), v_hbm.at[sl], v_v.at[sl]))
    plan.append(("w1", w1_hbm, w1_v))
    plan.append(("w2", w2_hbm, w2_v))
    for j in range(n_wo):
        sl = pl.ds(wo_off[j], _WO_CHUNKS[j])
        plan.append((("wo", j), wo_hbm.at[sl], wo_v.at[sl]))
    queue = [pltpu.make_async_copy(src, dst, sems.at[i]) for i, (_, src, dst) in enumerate(plan)]
    position = {name: i for i, (name, _, _) in enumerate(plan)}
    state = {"issued": 0, "waited": 0}

    def issue_upto(n):
        while state["issued"] < min(n, len(queue)):
            queue[state["issued"]].start()
            state["issued"] += 1

    def wait(name):
        while state["waited"] <= position[name]:
            queue[state["waited"]].wait()
            state["waited"] += 1
            issue_upto(state["waited"] + _WINDOW)

    small_sem = sems.at[len(queue)]
    small = [pltpu.make_async_copy(src, dst, small_sem)
             for src, dst in ((x_hbm, x_v), (gw_hbm, gw_v), (b1_hbm, b1_v), (b2_hbm, b2_v))]
    for c in small:
        c.start()
    issue_upto(_WINDOW)
    for c in small:
        c.wait()

    x4 = x_v[...]
    xf = x4.astype(f32)
    wait("wq")
    q = jnp.dot(x4, wq_v[...], preferred_element_type=f32)
    for j in range(_HQ):
        qp_s[pl.ds(j * 8, _B), :] = q[:, j * _DH:(j + 1) * _DH]
    zeros = jnp.zeros((8 - _REP, _DH), f32)
    for b in range(_B):
        for h in range(_HKV):
            i = b * _HKV + h
            qt_s[i, 0:_REP, :] = qp_s[pl.ds(h * _REP * 8 + b, _REP, stride=8), :]
            qt_s[i, _REP:8, :] = zeros

    scale = _DH ** -0.5

    def head(i, carry):
        qh = qt_s[i].astype(bf16)
        s = jax.lax.dot_general(qh, k_v[i], (((1,), (1,)), ((), ())),
                                preferred_element_type=f32) * scale
        m = jnp.max(s, axis=1, keepdims=True)
        p = jnp.exp(s - m)
        l = jnp.sum(p, axis=1, keepdims=True)
        o = jnp.dot(p.astype(bf16), v_v[i], preferred_element_type=f32)
        ot_s[pl.ds(pl.multiple_of(i * 8, 8), 8), :] = o / l
        return carry

    for c in range(n_kv):
        wait(("v", c))
        jax.lax.fori_loop(kv_off[c], kv_off[c] + _KV_CHUNKS[c], head, 0)

    gw = gw_v[...].astype(f32)
    gsum = jnp.zeros((_B, 1), f32)
    for t in range(_D // _LANES):
        gsum = gsum + jnp.sum(xf[:, t * _LANES:(t + 1) * _LANES] * gw[t:t + 1, :],
                              axis=1, keepdims=True)
    g = jax.nn.sigmoid(gsum)
    wait("w1")
    hpre = jnp.dot(x4, w1_v[...], preferred_element_type=f32)
    b1 = b1_v[...].astype(f32)
    hs = []
    for t in range(_F // _LANES):
        ht = hpre[:, t * _LANES:(t + 1) * _LANES] + b1[t:t + 1, :]
        r = jnp.where(ht > 0, ht, 0.0)
        hs.append((r * r).astype(bf16))
    hh = jnp.concatenate(hs, axis=1)
    wait("w2")
    mlp = jnp.dot(hh, w2_v[...], preferred_element_type=f32)
    b2 = b2_v[...].astype(f32)
    mlp = mlp + jnp.concatenate([b2[t:t + 1, :] for t in range(_D // _LANES)], axis=1)
    mix_b = (1.0 - g) * mlp

    acc = jnp.zeros((_B, _D), f32)
    for j in range(n_wo):
        tiles = []
        for t in range(wo_off[j] // _DH, (wo_off[j] + _WO_CHUNKS[j]) // _DH):
            h, r = t // _REP, t % _REP
            tiles.append(ot_s[pl.ds(8 * h + r, _B, stride=8 * _HKV), :].astype(bf16))
        lhs = tiles[0] if len(tiles) == 1 else jnp.concatenate(tiles, axis=1)
        wait(("wo", j))
        acc = acc + jnp.dot(lhs, wo_v[pl.ds(wo_off[j], _WO_CHUNKS[j]), :],
                            preferred_element_type=f32)
    o_ref[...] = (g * acc + mix_b).astype(o_ref.dtype)


def _kernel(*refs):
    n_sems = 1 + 2 * len(_KV_CHUNKS) + 2 + len(_WO_CHUNKS) + 1

    def scoped(sems):
        _body(*refs, sems)

    pl.run_scoped(scoped, pltpu.SemaphoreType.DMA((n_sems,)))


@jax.jit
def pallas_gated_mix__gqa_block_cached__dense_activation_squared_relu__decode_kernel(
    A_x: jax.Array,
    A_k_cache: jax.Array,
    A_v_cache: jax.Array,
    A_wq: jax.Array,
    A_wo: jax.Array,
    B_x: jax.Array,
    B_w1: jax.Array,
    B_b1: jax.Array,
    B_w2: jax.Array,
    B_b2: jax.Array,
    gate_w: jax.Array,
):
    del B_x
    f32, bf16 = jnp.float32, jnp.bfloat16
    hbm = pl.BlockSpec(memory_space=pltpu.HBM)
    out = pl.pallas_call(
        _kernel,
        in_specs=[hbm] * 10,
        out_specs=pl.BlockSpec(memory_space=pltpu.VMEM),
        out_shape=jax.ShapeDtypeStruct((_B, _D), bf16),
        scratch_shapes=[
            pltpu.VMEM((_B, _D), bf16),
            pltpu.VMEM((_F // _LANES, _LANES), bf16),
            pltpu.VMEM((_D // _LANES, _LANES), bf16),
            pltpu.VMEM((_D // _LANES, _LANES), bf16),
            pltpu.VMEM((_D, _HQ * _DH), bf16),
            pltpu.VMEM((_HQ * _DH, _D), bf16),
            pltpu.VMEM((_D, _F), bf16),
            pltpu.VMEM((_F, _D), bf16),
            pltpu.VMEM((_NBH, _SK, _DH), bf16),
            pltpu.VMEM((_NBH, _SK, _DH), bf16),
            pltpu.VMEM((_HQ * 8 + 8, _DH), f32),
            pltpu.VMEM((_NBH, 8, _DH), f32),
            pltpu.VMEM((_NBH * 8 + 64, _DH), f32),
        ],
        compiler_params=pltpu.CompilerParams(vmem_limit_bytes=100 * 1024 * 1024),
    )(
        A_x.reshape(_B, _D),
        A_k_cache.reshape(_NBH, _SK, _DH),
        A_v_cache.reshape(_NBH, _SK, _DH),
        A_wq,
        A_wo,
        B_w1,
        B_b1.reshape(_F // _LANES, _LANES),
        B_w2,
        B_b2.reshape(_D // _LANES, _LANES),
        gate_w.reshape(_D // _LANES, _LANES),
    )
    return out.reshape(_B, 1, _D)
```

```python
import jax
import jax.numpy as jnp
import jax.experimental.pallas as pl
import jax.experimental.pallas.tpu as pltpu

_B, _D = 4, 512
_HQ, _HKV, _SK, _DH = 32, 8, 4096, 128
_REP = _HQ // _HKV
_F = 1792
_NBH = _B * _HKV
_LANES = 128

_KV_CHUNKS = (4, 4, 4, 4, 4, 4, 4, 4)
_WO_CHUNKS = (1024, 1024, 1024, 512, 256, 128, 128)
_WINDOW = 4


def _offsets(sizes):
    return [sum(sizes[:j]) for j in range(len(sizes))]


def _body(x_hbm, k_hbm, v_hbm, wq_hbm, wo_hbm, w1_hbm, b1_hbm, w2_hbm, b2_hbm, gw_hbm,
          o_ref,
          x_v, b1_v, b2_v, gw_v, wq_v, wo_v, w1_v, w2_v, k_v, v_v, qt_s, ot_s,
          sems):
    f32, bf16 = jnp.float32, jnp.bfloat16
    n_kv, n_wo = len(_KV_CHUNKS), len(_WO_CHUNKS)
    kv_off, wo_off = _offsets(_KV_CHUNKS), _offsets(_WO_CHUNKS)

    plan = [("wq", wq_hbm, wq_v)]
    for c in range(n_kv):
        sl = pl.ds(kv_off[c], _KV_CHUNKS[c])
        plan.append((("k", c), k_hbm.at[sl], k_v.at[sl]))
        plan.append((("v", c), v_hbm.at[sl], v_v.at[sl]))
    plan.append(("w1", w1_hbm, w1_v))
    plan.append(("w2", w2_hbm, w2_v))
    for j in range(n_wo):
        sl = pl.ds(wo_off[j], _WO_CHUNKS[j])
        plan.append((("wo", j), wo_hbm.at[sl], wo_v.at[sl]))
    queue = [pltpu.make_async_copy(src, dst, sems.at[i]) for i, (_, src, dst) in enumerate(plan)]
    position = {name: i for i, (name, _, _) in enumerate(plan)}
    state = {"issued": 0, "waited": 0}

    def issue_upto(n):
        while state["issued"] < min(n, len(queue)):
            queue[state["issued"]].start()
            state["issued"] += 1

    def wait(name):
        while state["waited"] <= position[name]:
            queue[state["waited"]].wait()
            state["waited"] += 1
            issue_upto(state["waited"] + _WINDOW)

    small_sem = sems.at[len(queue)]
    small = [pltpu.make_async_copy(src, dst, small_sem)
             for src, dst in ((x_hbm, x_v), (gw_hbm, gw_v), (b1_hbm, b1_v), (b2_hbm, b2_v))]
    for c in small:
        c.start()
    issue_upto(_WINDOW)
    for c in small:
        c.wait()

    x4 = x_v[...]
    xf = x4.astype(f32)
    wait("wq")
    q = jnp.dot(x4, wq_v[...], preferred_element_type=f32)
    qt_s[...] = jnp.zeros(qt_s.shape, f32)
    for j in range(_HQ):
        h, r = j // _REP, j % _REP
        for b in range(_B):
            qt_s[b * _HKV + h, r:r + 1, :] = q[b:b + 1, j * _DH:(j + 1) * _DH]

    scale = _DH ** -0.5

    def head(i, carry):
        qh = qt_s[i].astype(bf16)
        s = jax.lax.dot_general(qh, k_v[i], (((1,), (1,)), ((), ())),
                                preferred_element_type=f32) * scale
        m = jnp.max(s, axis=1, keepdims=True)
        p = jnp.exp(s - m)
        l = jnp.sum(p, axis=1, keepdims=True)
        o = jnp.dot(p.astype(bf16), v_v[i], preferred_element_type=f32)
        o = o / l
        b, h = i // _HKV, i % _HKV
        for r in range(_REP):
            ot_s[h * _REP + r, pl.ds(b, 1), :] = o[r:r + 1, :]
        return carry

    for c in range(n_kv):
        wait(("v", c))
        jax.lax.fori_loop(kv_off[c], kv_off[c] + _KV_CHUNKS[c], head, 0)

    gw = gw_v[...].astype(f32)
    gsum = jnp.zeros((_B, 1), f32)
    for t in range(_D // _LANES):
        gsum = gsum + jnp.sum(xf[:, t * _LANES:(t + 1) * _LANES] * gw[t:t + 1, :],
                              axis=1, keepdims=True)
    g = jax.nn.sigmoid(gsum)
    wait("w1")
    hpre = jnp.dot(x4, w1_v[...], preferred_element_type=f32)
    b1 = b1_v[...].astype(f32)
    hs = []
    for t in range(_F // _LANES):
        ht = hpre[:, t * _LANES:(t + 1) * _LANES] + b1[t:t + 1, :]
        r = jnp.where(ht > 0, ht, 0.0)
        hs.append((r * r).astype(bf16))
    hh = jnp.concatenate(hs, axis=1)
    wait("w2")
    mlp = jnp.dot(hh, w2_v[...], preferred_element_type=f32)
    b2 = b2_v[...].astype(f32)
    mlp = mlp + jnp.concatenate([b2[t:t + 1, :] for t in range(_D // _LANES)], axis=1)
    mix_b = (1.0 - g) * mlp

    acc = jnp.zeros((_B, _D), f32)
    for j in range(n_wo):
        tiles = []
        for t in range(wo_off[j] // _DH, (wo_off[j] + _WO_CHUNKS[j]) // _DH):
            tiles.append(ot_s[t, 0:_B, :].astype(bf16))
        lhs = tiles[0] if len(tiles) == 1 else jnp.concatenate(tiles, axis=1)
        wait(("wo", j))
        acc = acc + jnp.dot(lhs, wo_v[pl.ds(wo_off[j], _WO_CHUNKS[j]), :],
                            preferred_element_type=f32)
    o_ref[...] = (g * acc + mix_b).astype(o_ref.dtype)


def _kernel(*refs):
    n_sems = 1 + 2 * len(_KV_CHUNKS) + 2 + len(_WO_CHUNKS) + 1

    def scoped(sems):
        _body(*refs, sems)

    pl.run_scoped(scoped, pltpu.SemaphoreType.DMA((n_sems,)))


@jax.jit
def pallas_gated_mix__gqa_block_cached__dense_activation_squared_relu__decode_kernel(
    A_x: jax.Array,
    A_k_cache: jax.Array,
    A_v_cache: jax.Array,
    A_wq: jax.Array,
    A_wo: jax.Array,
    B_x: jax.Array,
    B_w1: jax.Array,
    B_b1: jax.Array,
    B_w2: jax.Array,
    B_b2: jax.Array,
    gate_w: jax.Array,
):
    del B_x
    f32, bf16 = jnp.float32, jnp.bfloat16
    hbm = pl.BlockSpec(memory_space=pltpu.HBM)
    out = pl.pallas_call(
        _kernel,
        in_specs=[hbm] * 10,
        out_specs=pl.BlockSpec(memory_space=pltpu.VMEM),
        out_shape=jax.ShapeDtypeStruct((_B, _D), bf16),
        scratch_shapes=[
            pltpu.VMEM((_B, _D), bf16),
            pltpu.VMEM((_F // _LANES, _LANES), bf16),
            pltpu.VMEM((_D // _LANES, _LANES), bf16),
            pltpu.VMEM((_D // _LANES, _LANES), bf16),
            pltpu.VMEM((_D, _HQ * _DH), bf16),
            pltpu.VMEM((_HQ * _DH, _D), bf16),
            pltpu.VMEM((_D, _F), bf16),
            pltpu.VMEM((_F, _D), bf16),
            pltpu.VMEM((_NBH, _SK, _DH), bf16),
            pltpu.VMEM((_NBH, _SK, _DH), bf16),
            pltpu.VMEM((_NBH, 8, _DH), f32),
            pltpu.VMEM((_HQ, 8, _DH), f32),
        ],
        compiler_params=pltpu.CompilerParams(vmem_limit_bytes=100 * 1024 * 1024),
    )(
        A_x.reshape(_B, _D),
        A_k_cache.reshape(_NBH, _SK, _DH),
        A_v_cache.reshape(_NBH, _SK, _DH),
        A_wq,
        A_wo,
        B_w1,
        B_b1.reshape(_F // _LANES, _LANES),
        B_w2,
        B_b2.reshape(_D // _LANES, _LANES),
        gate_w.reshape(_D // _LANES, _LANES),
    )
    return out.reshape(_B, 1, _D)
```
